```python
import jax
import jax.numpy as jnp

def _softmax(x, axis=-1):
    return jax.nn.softmax(x, axis=axis)
def _gelu(x):
    return jax.nn.gelu(x, approximate=True)
def _silu(x):
    return jax.nn.silu(x)
def _sigmoid(x):
    return jax.nn.sigmoid(x)
def _layernorm(x, axis=-1, eps=1e-5):
    m = jnp.mean(x, axis=axis, keepdims=True)
    v = jnp.var(x, axis=axis, keepdims=True)
    return (x - m) / jnp.sqrt(v + eps)
def _scatter_add(tgt, idx, src, axis=0):
    return tgt.at[idx].add(src)
def _segment_sum(src, seg, n):
    return jax.ops.segment_sum(src, seg, n)
class _Rng:
    def __init__(self, key):
        self._k = key
    def _next(self):
        self._k, sub = jax.random.split(self._k)
        return sub
    def normal(self, shape):
        return jax.random.normal(self._next(), shape, dtype=jnp.bfloat16)
    def randint(self, lo, hi, shape):
        return jax.random.randint(self._next(), shape, lo, hi, dtype=jnp.int32)
    def uniform(self, shape, lo=0.0, hi=1.0):
        return jax.random.uniform(self._next(), shape, jnp.bfloat16, lo, hi)
    def permutation(self, n):
        return jax.random.permutation(self._next(), n)


kernel_name = 'recurrent_scan__compressed_kv_cla__moe_arch_mod__decode'

def setup_inputs():
    _rng = _Rng(jax.random.key(int.from_bytes(__import__("os").urandom(4), "little")))
    _w = (lambda a: (lambda t: t.astype(jnp.bfloat16) if jnp.issubdtype(t.dtype, jnp.floating) else t)(jnp.asarray(a)))
    def _A_setup():
        B, H, Sq, Sk, D, M = 4, 32, 1, 4096, 128, 576
        Dc = 4 * D
        return {
            "x": _w((lambda *s: _rng.normal(s) * 0.05)(B, Sq, M)),
            "c_kv": _w((lambda *s: _rng.normal(s) * 0.05)(B, Sk, Dc)),
            "w_q": _w((lambda *s: _rng.normal(s) * 0.05)(M, H, D) * (M ** -0.5)),
            "w_uk": _w((lambda *s: _rng.normal(s) * 0.05)(Dc, H, D) * (Dc ** -0.5)),
            "w_uv": _w((lambda *s: _rng.normal(s) * 0.05)(Dc, H, D) * (Dc ** -0.5)),
            "w_o": _w((lambda *s: _rng.normal(s) * 0.05)(H, D, M) * ((H * D) ** -0.5)),
        }
    _A_in = _A_setup()

    def _B_setup():
        B, S, D, F, C = 4, 1, 576, 4608, 1
        return {
            "x": _w((lambda *s: _rng.normal(s) * 0.05)(B, S, D)),
            "w_r": _w((lambda *s: _rng.normal(s) * 0.05)(D)),
            "w_gate": _w((lambda *s: _rng.normal(s) * 0.05)(D, F)),
            "w_up": _w((lambda *s: _rng.normal(s) * 0.05)(D, F)),
            "w_down": _w((lambda *s: _rng.normal(s) * 0.05)(F, D)),
        }
    _B_in = _B_setup()

    return {
        "A_x": _A_in["x"],
        "A_c_kv": _A_in["c_kv"],
        "A_w_q": _A_in["w_q"],
        "A_w_uk": _A_in["w_uk"],
        "A_w_uv": _A_in["w_uv"],
        "A_w_o": _A_in["w_o"],
        "B_x": _B_in["x"],
        "B_w_r": _B_in["w_r"],
        "B_w_gate": _B_in["w_gate"],
        "B_w_up": _B_in["w_up"],
        "B_w_down": _B_in["w_down"],
    }

def reference(A_x, A_c_kv, A_w_q, A_w_uk, A_w_uv, A_w_o, B_x, B_w_r, B_w_gate, B_w_up, B_w_down):
    def _A_ref(x, c_kv, w_q, w_uk, w_uv, w_o):
        B, Sq, M = x.shape[0], x.shape[1], x.shape[2]
        Sk = c_kv.shape[1]
        H, D = w_q.shape[1], w_q.shape[2]
        q = jnp.einsum("bqm,mhd->bhqd", x, w_q)
        k = jnp.einsum("bkc,chd->bhkd", c_kv, w_uk)
        v = jnp.einsum("bkc,chd->bhkd", c_kv, w_uv)
        scores = jnp.einsum("bhqd,bhkd->bhqk", q, k) * (D ** -0.5)
        off = Sk - Sq
        qi = jnp.arange(Sq)[:, None]
        kj = jnp.arange(Sk)[None, :]
        cmask = kj <= (qi + off)
        scores = jnp.where(cmask[None, None], scores, -1e9)
        p = _softmax(scores, axis=-1)
        ctx = jnp.einsum("bhqk,bhkd->bhqd", p, v)
        return jnp.einsum("bhqd,hdm->bqm", ctx, w_o)

    def _B_ref(x, w_r, w_gate, w_up, w_down):
        B, S, D = x.shape
        C = 1
        r = x @ w_r
        idx = jnp.argsort(-r, axis=-1)[:, :C]
        idx_e = jnp.repeat(idx.reshape(B, C, 1), D, axis=2)
        x_sel = jnp.take_along_axis(x, idx_e, axis=1)
        g = _silu(x_sel @ w_gate)
        u = x_sel @ w_up
        y = (g * u) @ w_down
        r_sel = _sigmoid(jnp.take_along_axis(r, idx, axis=1))
        y = y * r_sel.reshape(B, C, 1)
        b_off = (jnp.arange(B) * S).reshape(B, 1)
        flat_idx = (idx + b_off).reshape(B * C)
        zero = (x * 0.0).reshape(B * S, D)
        upd = _scatter_add(zero, flat_idx, y.reshape(B * C, D), axis=0)
        return x + upd.reshape(B, S, D)

    x = A_x
    xn = _layernorm(x, axis=-1)
    s = _A_ref(xn, A_c_kv, A_w_q, A_w_uk, A_w_uv, A_w_o)
    g = _silu(_B_ref(xn, B_w_r, B_w_gate, B_w_up, B_w_down))
    return x + s * g
```

```python
import jax
import jax.numpy as jnp
import jax.experimental.pallas as pl
import jax.experimental.pallas.tpu as pltpu

_LANES = 128
_KV_CHUNK = 1024
_FF_CHUNK = 512
_NN = (((1,), (0,)), ((), ()))
_NT = (((1,), (1,)), ((), ()))


def _dot(a, b, dims):
    return jax.lax.dot_general(a, b, dims, preferred_element_type=jnp.float32)


def _iota(shape, dim):
    return jax.lax.broadcasted_iota(jnp.int32, shape, dim)


def _one_hot(cond):
    return jnp.where(cond, 1.0, 0.0).astype(jnp.bfloat16)


def _kernel(
    x_hbm, ckv_hbm, wq_hbm, wuk_hbm, wuv_hbm, wo_hbm, wr_hbm, wg_hbm, wu_hbm, wd_hbm,
    o_ref,
    x_buf, wr_buf, ckv_buf, wq_buf, wuk_buf, wuv_buf, wo_buf, wg_buf, wu_buf, wd_buf,
    z_buf, qa_buf, s_buf, lat_buf, hid_buf,
    small_sem, a_sem, kv_sem, b_sem, up_sem, down_sem,
):
    f32, bf16, u32 = jnp.float32, jnp.bfloat16, jnp.uint32
    batch, model = x_buf.shape
    _, seq, latent = ckv_buf.shape
    pairs, _, head_dim = wq_buf.shape
    heads = 2 * pairs
    hidden = wg_buf.shape[1]
    rows = batch * heads
    kv_chunks = seq // _KV_CHUNK
    ff_chunks = hidden // _FF_CHUNK

    def pair_copy(hbm, buf, sem, i):
        return pltpu.make_async_copy(hbm.bitcast(u32).at[:, i], buf.at[i], sem)

    def wq_copy(i):
        return pair_copy(wq_hbm, wq_buf, a_sem.at[0, i], i)

    def wuk_copy(i):
        return pair_copy(wuk_hbm, wuk_buf, a_sem.at[1, i], i)

    def kv_copy(b, j):
        keys = pl.ds(pl.multiple_of(j * _KV_CHUNK, _KV_CHUNK), _KV_CHUNK)
        return pltpu.make_async_copy(
            ckv_hbm.at[b, keys], ckv_buf.at[b, keys], kv_sem.at[b, j])

    def wuv_copy(i):
        return pair_copy(wuv_hbm, wuv_buf, b_sem.at[0, i], i)

    def wo_copy(i):
        return pltpu.make_async_copy(wo_hbm.at[i], wo_buf.at[i], b_sem.at[1, i])

    def ff_cols(j):
        return pl.ds(pl.multiple_of(j * _FF_CHUNK, _FF_CHUNK), _FF_CHUNK)

    def ff_copy(hbm, buf, sem, j):
        return pltpu.make_async_copy(hbm.at[:, ff_cols(j)], buf.at[:, ff_cols(j)], sem)

    def wg_copy(j):
        return ff_copy(wg_hbm, wg_buf, up_sem.at[0, j], j)

    def wu_copy(j):
        return ff_copy(wu_hbm, wu_buf, up_sem.at[1, j], j)

    def wd_copy(j):
        return ff_copy(wd_hbm, wd_buf, down_sem.at[j], j)

    x_copy = pltpu.make_async_copy(x_hbm, x_buf, small_sem.at[0])
    wr_copy = pltpu.make_async_copy(wr_hbm, wr_buf, small_sem.at[1])

    x_copy.start()
    wr_copy.start()

    @pl.loop(0, pairs)
    def _(i):
        wq_copy(i).start()
        wuk_copy(i).start()

    for b in range(batch):
        for j in range(kv_chunks):
            kv_copy(b, j).start()

    spread = _one_hot(_iota((_LANES, 2 * _LANES), 1) // 2 == _iota((_LANES, 2 * _LANES), 0))
    r, c = _iota((rows, rows), 0), _iota((rows, rows), 1)
    by_batch = _one_hot(c == (r % heads) * batch + r // heads)
    by_head = _one_hot(r == (c % heads) * batch + c // heads)

    def own_head(shape):
        return (_iota(shape, 0) // batch) % 2 == _iota(shape, 1) % 2

    def spread_lanes(v):
        k = v.shape[1]
        parts = []
        for k0 in range(0, k, _LANES):
            w = min(_LANES, k - k0)
            parts.append(_dot(v[:, k0:k0 + w], spread[:w, :2 * w], _NN))
        out = jnp.concatenate(parts, axis=1)
        return jnp.where(own_head(out.shape), out, 0.0)

    x_copy.wait()
    wr_copy.wait()
    x = x_buf[...].astype(f32)
    mean = jnp.mean(x, axis=-1, keepdims=True)
    var = jnp.mean(jnp.square(x - mean), axis=-1, keepdims=True)
    xn_bf = ((x - mean) / jnp.sqrt(var + 1e-5)).astype(bf16)
    xn = xn_bf.astype(f32)
    w_r = wr_buf[...].astype(f32).reshape(1, model)
    route = jax.nn.sigmoid(jnp.sum(xn * w_r, axis=-1, keepdims=True))
    xn_pair = spread_lanes(jnp.concatenate([xn, xn], axis=0).astype(bf16)).astype(bf16)

    @pl.loop(0, pairs)
    def _(i):
        wq_copy(i).wait()
        q = _dot(xn_pair, pltpu.bitcast(wq_buf[i], bf16), _NN)
        wuk_copy(i).wait()
        z = _dot(q.astype(bf16), pltpu.bitcast(wuk_buf[i], bf16), _NT)
        z = jnp.where(own_head(z.shape), z * head_dim ** -0.5, 0.0)
        z_buf[pl.ds(pl.multiple_of(i * 2 * batch, 2 * batch), 2 * batch), :] = z

    @pl.loop(0, pairs)
    def _(i):
        wuv_copy(i).start()
        wo_copy(i).start()

    for k0 in range(0, latent, _LANES):
        part = _dot(z_buf[:, 2 * k0:2 * (k0 + _LANES)].astype(bf16), spread, _NT)
        qa_buf[:, k0:k0 + _LANES] = _dot(by_batch, part.astype(bf16), _NN).astype(bf16)

    @pl.loop(0, batch)
    def _(b):
        head_rows = pl.ds(pl.multiple_of(b * heads, heads), heads)
        q_abs = qa_buf[head_rows, :]

        def score_chunk(j, top):
            keys = pl.ds(pl.multiple_of(j * _KV_CHUNK, _KV_CHUNK), _KV_CHUNK)
            kv_copy(b, j).wait()
            s = _dot(q_abs, ckv_buf[b, keys, :], _NT)
            s_buf[:, keys] = s
            for k0 in range(0, _KV_CHUNK, _LANES):
                top = jnp.maximum(top, s[:, k0:k0 + _LANES])
            return top

        top = jax.lax.fori_loop(
            0, kv_chunks, score_chunk, jnp.full((heads, _LANES), -jnp.inf, f32))
        top = jnp.max(top, axis=-1, keepdims=True)

        def mix_chunk(j, carry):
            total, acc = carry
            keys = pl.ds(pl.multiple_of(j * _KV_CHUNK, _KV_CHUNK), _KV_CHUNK)
            p = jnp.exp(s_buf[:, keys] - top)
            for k0 in range(0, _KV_CHUNK, _LANES):
                total = total + p[:, k0:k0 + _LANES]
            return total, acc + _dot(p.astype(bf16), ckv_buf[b, keys, :], _NN)

        total, acc = jax.lax.fori_loop(
            0, kv_chunks, mix_chunk,
            (jnp.zeros((heads, _LANES), f32), jnp.zeros((heads, latent), f32)))
        lat_buf[head_rows, :] = (acc / jnp.sum(total, axis=-1, keepdims=True)).astype(bf16)

    @pl.loop(0, ff_chunks)
    def _(j):
        wg_copy(j).start()
        wu_copy(j).start()

    @pl.loop(0, ff_chunks)
    def _(j):
        wd_copy(j).start()

    z_buf[...] = spread_lanes(_dot(by_head, lat_buf[...], _NN).astype(bf16))

    def project_pair(i, acc):
        lat = z_buf[pl.ds(pl.multiple_of(i * 2 * batch, 2 * batch), 2 * batch), :]
        wuv_copy(i).wait()
        ctx = _dot(lat.astype(bf16), pltpu.bitcast(wuv_buf[i], bf16), _NN)
        wo_copy(i).wait()
        return acc + _dot(ctx.astype(bf16), wo_buf[i], _NT)

    acc = jax.lax.fori_loop(0, pairs, project_pair, jnp.zeros((2 * batch, 2 * model), f32))
    attn = acc[:batch, :model] + acc[batch:, model:]

    @pl.loop(0, ff_chunks)
    def _(j):
        wg_copy(j).wait()
        gate = _dot(xn_bf, wg_buf[:, ff_cols(j)], _NN)
        wu_copy(j).wait()
        up = _dot(xn_bf, wu_buf[:, ff_cols(j)], _NN)
        hid_buf[:, ff_cols(j)] = jax.nn.silu(gate) * up

    def down_chunk(j, y):
        wd_copy(j).wait()
        return y + _dot(hid_buf[:, ff_cols(j)].astype(bf16), wd_buf[:, ff_cols(j)], _NT)

    y = jax.lax.fori_loop(0, ff_chunks, down_chunk, jnp.zeros((batch, model), f32))
    gate = jax.nn.silu(xn + (xn * 0.0 + y * route))
    o_ref[...] = (x + attn * gate).astype(o_ref.dtype)


@jax.jit
def pallas_recurrent_scan__compressed_kv_cla__moe_arch_mod__decode_kernel(
    A_x: jax.Array,
    A_c_kv: jax.Array,
    A_w_q: jax.Array,
    A_w_uk: jax.Array,
    A_w_uv: jax.Array,
    A_w_o: jax.Array,
    B_x: jax.Array,
    B_w_r: jax.Array,
    B_w_gate: jax.Array,
    B_w_up: jax.Array,
    B_w_down: jax.Array,
):
    del B_x
    batch, _, model = A_x.shape
    _, seq, latent = A_c_kv.shape
    _, heads, head_dim = A_w_q.shape
    hidden = B_w_gate.shape[1]
    pairs = heads // 2
    f32, bf16, u32 = jnp.float32, jnp.bfloat16, jnp.uint32
    in_hbm = pl.BlockSpec(memory_space=pl.ANY)
    dma = pltpu.SemaphoreType.DMA

    out = pl.pallas_call(
        _kernel,
        in_specs=[in_hbm] * 10,
        out_specs=pl.BlockSpec(memory_space=pltpu.VMEM),
        out_shape=jax.ShapeDtypeStruct((batch, model), A_x.dtype),
        scratch_shapes=[
            pltpu.VMEM((batch, model), bf16),
            pltpu.VMEM((model,), bf16),
            pltpu.VMEM((batch, seq, latent), bf16),
            pltpu.VMEM((pairs, model, head_dim), u32),
            pltpu.VMEM((pairs, latent, head_dim), u32),
            pltpu.VMEM((pairs, latent, head_dim), u32),
            pltpu.VMEM((pairs, 2 * model, head_dim), bf16),
            pltpu.VMEM((model, hidden), bf16),
            pltpu.VMEM((model, hidden), bf16),
            pltpu.VMEM((model, hidden), bf16),
            pltpu.VMEM((batch * heads, 2 * latent), f32),
            pltpu.VMEM((batch * heads, latent), bf16),
            pltpu.VMEM((heads, seq), f32),
            pltpu.VMEM((batch * heads, latent), bf16),
            pltpu.VMEM((batch, hidden), f32),
            dma((2,)),
            dma((2, pairs)),
            dma((batch, seq // _KV_CHUNK)),
            dma((2, pairs)),
            dma((2, hidden // _FF_CHUNK)),
            dma((hidden // _FF_CHUNK,)),
        ],
        compiler_params=pltpu.CompilerParams(
            vmem_limit_bytes=100 * 1024 * 1024,
            disable_semaphore_checks=True,
        ),
    )(
        A_x.reshape(batch, model),
        A_c_kv,
        A_w_q,
        A_w_uk,
        A_w_uv,
        jnp.transpose(A_w_o, (0, 2, 1)).reshape(pairs, 2 * model, head_dim),
        B_w_r,
        B_w_gate,
        B_w_up,
        B_w_down.T,
    )
    return out.reshape(A_x.shape)
```

```python
import functools

import jax
import jax.numpy as jnp
import jax.experimental.pallas as pl
import jax.experimental.pallas.tpu as pltpu

_LANES = 128
_ROWS = 16
_WORDS = 32
_REGIONS = (2, 4)
_UNIT = 16
_TRIPLES = 5
_LAG = 4
_GROUPS = 4
_KEYS = 512
_NN = (((1,), (0,)), ((), ()))
_NT = (((1,), (1,)), ((), ()))


def _dot(a, b, dims):
    return jax.lax.dot_general(a, b, dims, preferred_element_type=jnp.float32)


def _iota(shape, dim):
    return jax.lax.broadcasted_iota(jnp.int32, shape, dim)


def _one_hot(cond):
    return jnp.where(cond, 1.0, 0.0).astype(jnp.bfloat16)


def _wait_filled(dst, sem):
    pltpu.make_async_copy(dst, dst, sem).wait()


def _kernel(
    x_hbm, ckv_hbm, wq_hbm, wuk_hbm, wuv_hbm, wo_hbm, wr_hbm, wg_hbm, wu_hbm, wd_hbm,
    o_ref,
    x_buf, wr_buf, kv_buf, ff_buf, wq_buf, wuk_buf, wuv_buf, wo_buf,
    xn_buf, q_buf, wide_buf, qa_buf, s_buf, lat_buf, ctx_buf, y_buf,
    small_sem, w_sem, kv_sem, wo_sem, ff_sem,
):
    f32, bf16, u32 = jnp.float32, jnp.bfloat16, jnp.uint32
    batch, model = x_buf.shape
    _, heads, seq = s_buf.shape
    latent = kv_buf.shape[-1]
    head_dim = wq_buf.shape[-1]
    rows = batch * heads
    slots = heads // _GROUPS
    group_rows = slots * batch
    wide = slots * _LANES
    chunks = seq // _KEYS
    kv_pieces = _KEYS // _ROWS
    ff_pieces = model // _ROWS
    ff_blocks = wg_hbm.shape[-1] // latent
    head_words = model // 2
    regions = [(a, s) for a in range(_REGIONS[0]) for s in range(_REGIONS[1])]

    def words_copy(hbm, buf, sem, first, t):
        r = pl.ds(pl.multiple_of(first, _WORDS), _WORDS)
        return pltpu.make_async_copy(
            hbm.bitcast(u32).at[:, t & 3, r], buf.at[:, t & 3, r], sem)

    def weight_copy(hbm, buf, sem, t):
        return words_copy(hbm, buf, sem, (t >> 2) * _WORDS, t)

    def wo_copy(t):
        block, k = t >> 4, (t >> 2) & 3
        return words_copy(
            wo_hbm, wo_buf, wo_sem.at[block, k], k * head_words + block * _WORDS, t)

    def kv_copy(t):
        return pltpu.make_async_copy(
            ckv_hbm.at[t >> 7, :, t & 3, (t >> 2) & 31],
            kv_buf.at[pl.ds(2 * t, 2)], kv_sem.at[t >> 4])

    recip = -(-(1 << 16) // ff_pieces)
    assert all((n * recip) >> 16 == n // ff_pieces for n in range(ff_blocks * ff_pieces))

    def ff_copy(m, n):
        block = (n * recip) >> 16
        r = n - block * ff_pieces
        cols = pl.ds(pl.multiple_of(block * latent, latent), latent)
        return pltpu.make_async_copy(
            (wg_hbm, wu_hbm, wd_hbm)[m].at[r, :, cols],
            ff_buf.at[(3 * block + m) * ff_pieces + r], ff_sem.at[block])

    def units_of(buf):
        return buf.shape[1] * buf.shape[2] // (_WORDS * _UNIT)

    stream = [
        (functools.partial(weight_copy, wq_hbm, wq_buf, w_sem.at[0]), units_of(wq_buf)),
        (functools.partial(weight_copy, wuk_hbm, wuk_buf, w_sem.at[1]), units_of(wuk_buf)),
        (kv_copy, batch * chunks),
        (functools.partial(weight_copy, wuv_hbm, wuv_buf, w_sem.at[2]), units_of(wuv_buf)),
        (wo_copy, units_of(wo_buf)),
    ]
    ends = [sum(n for _, n in stream[:k + 1]) for k in range(len(stream))]
    wq_end, wuk_end, _, wuv_end, last_unit = ends
    triples = ff_blocks * ff_pieces
    cuts = sorted(ends + [triples // _TRIPLES, triples // _TRIPLES + 1])

    def burst(lo, hi, u):
        for cut in cuts:
            if lo < cut < hi:
                pl.when(u < cut)(lambda: burst(lo, cut, u))
                pl.when(u >= cut)(lambda: burst(cut, hi, u))
                return
        k = next(k for k, end in enumerate(ends) if lo < end)
        copy, units = stream[k]
        first = _UNIT * (u - (ends[k] - units))
        count = max(0, min(_TRIPLES, triples - _TRIPLES * lo))
        copy(first).start(priority=1)
        if count:
            @pl.loop(0, count)
            def _(i):
                for m in range(3):
                    ff_copy(m, _TRIPLES * u + i).start(priority=0)
                    copy(first + 1 + 3 * i + m).start(priority=1)
        if 1 + 3 * count < _UNIT:
            @pl.loop(1 + 3 * count, _UNIT)
            def _(i):
                copy(first + i).start(priority=1)

    queued = [0]

    def steps(n, body=None, carry=None):
        first = queued[0]
        queued[0] += n

        def step(i, carry):
            burst(first, first + n, first + i)
            return carry if body is None else body(i, carry)

        return step(0, carry) if n == 1 else jax.lax.fori_loop(0, n, step, carry)

    def queue_until(unit):
        unit = min(unit, last_unit)
        if unit > queued[0]:
            steps(unit - queued[0])

    def slab(buf, first, n):
        return buf[pl.ds(first, n)].reshape(n * _ROWS, latent)

    def head_group(buf, g):
        every = pl.ds(g, buf.shape[2] // _GROUPS, stride=_GROUPS)
        words = jnp.concatenate([buf[a, s, every, :] for a, s in regions], axis=0)
        return pltpu.bitcast(words, bf16)

    def rows_of(g):
        return pl.ds(pl.multiple_of(g * group_rows, group_rows), group_rows)

    x_copy = pltpu.make_async_copy(x_hbm, x_buf, small_sem.at[0])
    wr_copy = pltpu.make_async_copy(wr_hbm, wr_buf, small_sem.at[1])
    x_copy.start()
    wr_copy.start()
    queue_until(2)

    spread = _one_hot(_iota((_LANES, wide), 1) // slots == _iota((_LANES, wide), 0))

    def batch_major(row):
        g, slot = row // group_rows, (row // batch) % slots
        head = (slot // 2) * (2 * _GROUPS) + 2 * g + slot % 2
        return (row % batch) * heads + head

    by_batch = _one_hot(_iota((rows, rows), 0) == batch_major(_iota((rows, rows), 1)))
    by_group = _one_hot(_iota((rows, rows), 1) == batch_major(_iota((rows, rows), 0)))

    def own_slot(v):
        keep = (_iota(v.shape, 0) // batch) % slots == _iota(v.shape, 1) % slots
        return jnp.where(keep, v, 0.0).astype(bf16)

    y_buf[...] = jnp.zeros_like(y_buf)
    x_copy.wait()
    wr_copy.wait()
    x = x_buf[...].astype(f32)
    mean = jnp.mean(x, axis=-1, keepdims=True)
    var = jnp.mean(jnp.square(x - mean), axis=-1, keepdims=True)
    xn_bf = ((x - mean) / jnp.sqrt(var + 1e-5)).astype(bf16)
    xn = xn_bf.astype(f32)
    w_r = wr_buf[...].astype(f32).reshape(1, model)
    route = jax.nn.sigmoid(jnp.sum(xn * w_r, axis=-1, keepdims=True))
    xn_rows = jnp.concatenate([xn, xn], axis=0)
    xn_rows = jnp.concatenate([xn_rows] * (slots // 2), axis=0).astype(bf16)
    for k0 in range(0, model, _LANES):
        n = min(_LANES, model - k0)
        xn_buf[:, slots * k0:slots * (k0 + n)] = own_slot(
            _dot(xn_rows[:, k0:k0 + n], spread[:n, :slots * n], _NN))

    def ffn_block(j):
        _wait_filled(ff_buf.at[pl.ds(3 * j * ff_pieces, 3 * ff_pieces)], ff_sem.at[j])
        gate, up, down = (slab(ff_buf, (3 * j + m) * ff_pieces, ff_pieces) for m in range(3))
        hidden = jax.nn.silu(_dot(xn_bf, gate, _NN)) * _dot(xn_bf, up, _NN)
        y_buf[...] += _dot(hidden.astype(bf16), down, _NT)

    def query(g):
        q_buf[g] = _dot(xn_buf[...], head_group(wq_buf, g), _NN).astype(bf16)

    def absorb(g):
        z = _dot(q_buf[g], head_group(wuk_buf, g), _NT)
        wide_buf[rows_of(g), :] = own_slot(z * head_dim ** -0.5)

    queue_until(wq_end + _LAG - 2)
    ffn_block(0)
    queue_until(wq_end + _LAG)
    _wait_filled(wq_buf, w_sem.at[0])
    query(0)
    steps(_GROUPS - 1, lambda i, _: query(i + 1))
    queue_until(wuk_end + _LAG - 2)
    ffn_block(1)
    queue_until(wuk_end + _LAG)
    _wait_filled(wuk_buf, w_sem.at[1])
    pl.loop(0, _GROUPS // 2)(absorb)
    steps(1)
    pl.loop(_GROUPS // 2, _GROUPS)(absorb)
    for k in range(latent // _LANES):
        if k % 2 == 0:
            steps(1)
        part = _dot(wide_buf[:, k * wide:(k + 1) * wide], spread, _NT).astype(bf16)
        qa_buf[:, k * _LANES:(k + 1) * _LANES] = _dot(by_batch, part, _NN).astype(bf16)

    def attend(j, carry, new, old, top):
        new_top, total, acc = carry
        keys = pl.ds(pl.multiple_of(j * _KEYS, _KEYS), _KEYS)
        if old is not None:
            p = jnp.exp(s_buf[old % 2, :, keys] - top)
            for k0 in range(0, _KEYS, _LANES):
                total = total + p[:, k0:k0 + _LANES]
            values = slab(kv_buf, (old * chunks + j) * kv_pieces, kv_pieces)
            acc = acc + _dot(p.astype(bf16), values, _NN)
        if new is not None:
            u = new * chunks + j
            _wait_filled(kv_buf.at[pl.ds(u * kv_pieces, kv_pieces)], kv_sem.at[u])
            s = _dot(qa_buf[pl.ds(new * heads, heads), :],
                     slab(kv_buf, u * kv_pieces, kv_pieces), _NT)
            s_buf[new % 2, :, keys] = s
            for k0 in range(0, _KEYS, _LANES):
                new_top = jnp.maximum(new_top, s[:, k0:k0 + _LANES])
        return new_top, total, acc

    top = None
    for b in range(batch + 1):
        new = b if b < batch else None
        old = b - 1 if b > 0 else None
        chunk = functools.partial(attend, new=new, old=old, top=top)
        per = 2 if old is None else (chunks // 2 if new is None else 1)

        def some_chunks(i, carry, chunk=chunk, per=per):
            return jax.lax.fori_loop(i * per, (i + 1) * per, chunk, carry)

        new_top, total, acc = steps(chunks // per, chunk if per == 1 else some_chunks, (
            None if new is None else jnp.full((heads, _LANES), -jnp.inf, f32),
            None if old is None else jnp.zeros((heads, _LANES), f32),
            None if old is None else jnp.zeros((heads, latent), f32)))
        if old is not None:
            lat = acc / jnp.sum(total, axis=-1, keepdims=True)
            lat_buf[pl.ds(old * heads, heads), :] = lat.astype(bf16)
        if new is not None:
            top = jnp.max(new_top, axis=-1, keepdims=True)
            ffn_block(2 + b)

    def context(g):
        ctx = _dot(wide_buf[rows_of(g), :], head_group(wuv_buf, g), _NN)
        odd = _iota((2 * batch, head_dim), 0) >= batch
        for p in range(slots // 2):
            pair = ctx[2 * batch * p:2 * batch * (p + 1)]
            head = 2 * _GROUPS * p + 2 * g
            ctx_buf[head] = jnp.where(odd, 0.0, pair).astype(bf16)
            ctx_buf[head + 1] = jnp.where(odd, pair, 0.0).astype(bf16)

    steps(1)
    lat = _dot(by_group, lat_buf[...], _NN).astype(bf16)
    for k in range(latent // _LANES):
        wide_buf[:, k * wide:(k + 1) * wide] = own_slot(
            _dot(lat[:, k * _LANES:(k + 1) * _LANES], spread, _NN))
    steps(1)
    ffn_block(6)
    queue_until(wuv_end + _LAG)
    _wait_filled(wuv_buf, w_sem.at[2])
    pl.loop(0, _GROUPS // 2)(context)
    steps(1)
    pl.loop(_GROUPS // 2, _GROUPS)(context)

    def project(block, n, ks):
        def rows_at(k, block, n):
            return pl.ds(k * head_words + block * _WORDS, n * _WORDS)

        for k in ks:
            for b in range(block, block + n):
                _wait_filled(wo_buf.at[:, :, rows_at(k, b, 1)], wo_sem.at[b, k])
        ctx = jnp.concatenate(
            [ctx_buf[4 * i + k] for k in ks for i in range(len(regions))], axis=1)
        w_o = jnp.concatenate(
            [pltpu.bitcast(wo_buf[a, s, rows_at(k, block, n), :], bf16)
             for k in ks for a, s in regions], axis=1)
        return _dot(ctx, w_o, _NT)

    full = model // _LANES
    split = full * _LANES
    attn = []
    for i in range(full):
        queue_until(max(queued[0] + 1, wuv_end + 2 * (i + 1) + _LAG))
        if i == 0:
            ffn_block(7)
        if i == full - 1:
            ffn_block(8)
            gate = jax.nn.silu(xn + (xn * 0.0 + y_buf[...] * route))
        acc = project(2 * i, 2, range(4))
        attn.append(acc[:batch] + acc[batch:])
    assert queued[0] == last_unit and ff_blocks == 9
    attn = jnp.concatenate(attn, axis=1)
    o_ref[:, :split] = (x[:, :split] + attn * gate[:, :split]).astype(o_ref.dtype)
    acc = project(2 * full, 1, (0, 1, 2))
    acc = acc + project(2 * full, 1, (3,))
    attn = acc[:batch] + acc[batch:]
    o_ref[:, split:] = (x[:, split:] + attn * gate[:, split:]).astype(o_ref.dtype)


@jax.jit
def pallas_recurrent_scan__compressed_kv_cla__moe_arch_mod__decode_kernel(
    A_x: jax.Array,
    A_c_kv: jax.Array,
    A_w_q: jax.Array,
    A_w_uk: jax.Array,
    A_w_uv: jax.Array,
    A_w_o: jax.Array,
    B_x: jax.Array,
    B_w_r: jax.Array,
    B_w_gate: jax.Array,
    B_w_up: jax.Array,
    B_w_down: jax.Array,
):
    del B_x
    batch, _, model = A_x.shape
    _, seq, latent = A_c_kv.shape
    _, heads, head_dim = A_w_q.shape
    hidden = B_w_gate.shape[1]
    parts = _REGIONS[0] * _REGIONS[1]
    slots = heads // _GROUPS
    f32, bf16, u32 = jnp.float32, jnp.bfloat16, jnp.uint32
    vmem, dma = pltpu.VMEM, pltpu.SemaphoreType.DMA

    def by_region(w):
        return w.reshape(*_REGIONS, -1, head_dim)

    def by_piece(w):
        return w.reshape(model // _ROWS, _ROWS, hidden)

    def words(n):
        return vmem((*_REGIONS, n * heads // (2 * parts), head_dim), u32)

    out = pl.pallas_call(
        _kernel,
        in_specs=[pl.BlockSpec(memory_space=pl.ANY)] * 10,
        out_specs=pl.BlockSpec(memory_space=pltpu.VMEM),
        out_shape=jax.ShapeDtypeStruct((batch, model), A_x.dtype),
        scratch_shapes=[
            vmem((batch, model), bf16),
            vmem((model,), bf16),
            vmem((batch * seq // _ROWS, _ROWS, latent), bf16),
            vmem((3 * (hidden // latent) * (model // _ROWS), _ROWS, latent), bf16),
            words(model), words(latent), words(latent), words(model),
            vmem((slots * batch, slots * model), bf16),
            vmem((_GROUPS, slots * batch, head_dim), bf16),
            vmem((batch * heads, slots * latent), bf16),
            vmem((batch * heads, latent), bf16),
            vmem((2, heads, seq), f32),
            vmem((batch * heads, latent), bf16),
            vmem((heads, 2 * batch, head_dim), bf16),
            vmem((batch, model), f32),
            dma((2,)),
            dma((3,)),
            dma((batch * seq // _KEYS,)),
            dma((model // (2 * _WORDS), heads // parts)),
            dma((hidden // latent,)),
        ],
        compiler_params=pltpu.CompilerParams(
            vmem_limit_bytes=100 * 1024 * 1024,
            disable_semaphore_checks=True,
            disable_bounds_checks=True,
        ),
    )(
        A_x.reshape(batch, model),
        A_c_kv.reshape(batch, *_REGIONS, seq // (parts * _ROWS), _ROWS, latent),
        by_region(A_w_q),
        by_region(A_w_uk),
        by_region(A_w_uv),
        by_region(jnp.transpose(A_w_o, (0, 2, 1))),
        B_w_r,
        by_piece(B_w_gate),
        by_piece(B_w_up),
        by_piece(B_w_down.T),
    )
    return out.reshape(A_x.shape)
```

```python
import functools

import jax
import jax.numpy as jnp
import jax.experimental.pallas as pl
import jax.experimental.pallas.tpu as pltpu

_LANES = 128
_ROWS = 16
_WORDS = 32
_REGIONS = (2, 4)
_UNIT = 16
_TRIPLES = 5
_LAG = 4
_GROUPS = 4
_KEYS = 512
_NN = (((1,), (0,)), ((), ()))
_NT = (((1,), (1,)), ((), ()))


def _dot(a, b, dims):
    return jax.lax.dot_general(a, b, dims, preferred_element_type=jnp.float32)


def _iota(shape, dim):
    return jax.lax.broadcasted_iota(jnp.int32, shape, dim)


def _one_hot(cond):
    return jnp.where(cond, 1.0, 0.0).astype(jnp.bfloat16)


def _wait_filled(dst, sem):
    pltpu.make_async_copy(dst, dst, sem).wait()


def _kernel(
    x_hbm, ckv_hbm, wq_hbm, wuk_hbm, wuv_hbm, wo_hbm, wr_hbm, wg_hbm, wu_hbm, wd_hbm,
    o_ref,
    x_buf, wr_buf, kv_buf, ff_buf, wq_buf, wuk_buf, wuv_buf, wo_buf,
    xn_buf, q_buf, wide_buf, qa_buf, s_buf, lat_buf, ctx_buf, y_buf,
    small_sem, w_sem, kv_sem, wo_sem, ff_sem,
):
    f32, bf16, u32 = jnp.float32, jnp.bfloat16, jnp.uint32
    batch, model = x_buf.shape
    _, heads, seq = s_buf.shape
    latent = kv_buf.shape[-1]
    head_dim = wq_buf.shape[-1]
    rows = batch * heads
    slots = heads // _GROUPS
    group_rows = slots * batch
    wide = slots * _LANES
    chunks = seq // _KEYS
    kv_pieces = _KEYS // _ROWS
    ff_pieces = model // _ROWS
    ff_blocks = wg_hbm.shape[-1] // latent
    head_words = model // 2
    full_blocks = model // _LANES
    regions = [(a, s) for a in range(_REGIONS[0]) for s in range(_REGIONS[1])]
    assert (batch, heads, seq, latent, model, ff_blocks) == (4, 32, 4096, 512, 576, 9)

    def words_copy(hbm, buf, sem, s, first):
        r = pl.ds(pl.multiple_of(first, _WORDS), _WORDS)
        return pltpu.make_async_copy(hbm.bitcast(u32).at[:, s, r], buf.at[:, s, r], sem)

    def weight_copy(hbm, buf, sem, t):
        return words_copy(hbm, buf, sem, t & 3, (t >> 2) * _WORDS)

    def wo_copy(block, half, part):
        first = (part >> 2) * head_words + (2 * block + half) * _WORDS
        return words_copy(wo_hbm, wo_buf, wo_sem.at[block, part], part & 3, first)

    def kv_copy(t):
        return pltpu.make_async_copy(
            ckv_hbm.at[t >> 7, :, t & 3, (t >> 2) & 31],
            kv_buf.at[pl.ds(2 * t, 2)], kv_sem.at[t >> 4])

    recip = -(-(1 << 16) // ff_pieces)
    assert all((n * recip) >> 16 == n // ff_pieces for n in range(ff_blocks * ff_pieces))

    def ff_copy(m, n):
        block = (n * recip) >> 16
        r = n - block * ff_pieces
        cols = pl.ds(pl.multiple_of(block * latent, latent), latent)
        return pltpu.make_async_copy(
            (wg_hbm, wu_hbm, wd_hbm)[m].at[r, :, cols],
            ff_buf.at[(3 * block + m) * ff_pieces + r], ff_sem.at[block])

    def units_of(buf):
        return buf.shape[1] * buf.shape[2] // (_WORDS * _UNIT)

    stream = [
        (functools.partial(weight_copy, wq_hbm, wq_buf, w_sem.at[0]), units_of(wq_buf)),
        (functools.partial(weight_copy, wuk_hbm, wuk_buf, w_sem.at[1]), units_of(wuk_buf)),
        (kv_copy, batch * chunks),
        (functools.partial(weight_copy, wuv_hbm, wuv_buf, w_sem.at[2]), units_of(wuv_buf)),
        (lambda t: wo_copy(full_blocks, 0, t), 1),
        (lambda t: wo_copy(t >> 5, t & 1, (t >> 1) & 15), 2 * full_blocks),
    ]
    ends = [sum(n for _, n in stream[:k + 1]) for k in range(len(stream))]
    wq_end, wuk_end, _, wuv_end, narrow_end, last_unit = ends
    triples = ff_blocks * ff_pieces
    cuts = sorted(ends + [triples // _TRIPLES, triples // _TRIPLES + 1])

    def burst(lo, hi, u):
        for cut in cuts:
            if lo < cut < hi:
                pl.when(u < cut)(lambda: burst(lo, cut, u))
                pl.when(u >= cut)(lambda: burst(cut, hi, u))
                return
        k = next(k for k, end in enumerate(ends) if lo < end)
        copy, units = stream[k]
        first = _UNIT * (u - (ends[k] - units))
        count = max(0, min(_TRIPLES, triples - _TRIPLES * lo))
        copy(first).start(priority=1)
        if count:
            @pl.loop(0, count)
            def _(i):
                for m in range(3):
                    ff_copy(m, _TRIPLES * u + i).start(priority=0)
                    copy(first + 1 + 3 * i + m).start(priority=1)
        if 1 + 3 * count < _UNIT:
            @pl.loop(1 + 3 * count, _UNIT)
            def _(i):
                copy(first + i).start(priority=1)

    queued = [0]

    def steps(n, body=None, carry=None):
        first = queued[0]
        queued[0] += n

        def step(i, carry):
            burst(first, first + n, first + i)
            return carry if body is None else body(i, carry)

        return step(0, carry) if n == 1 else jax.lax.fori_loop(0, n, step, carry)

    def queue_until(unit):
        unit = min(unit, last_unit)
        if unit > queued[0]:
            steps(unit - queued[0])

    def slab(buf, first, n):
        return buf[pl.ds(first, n)].reshape(n * _ROWS, latent)

    def head_group(buf, g):
        every = pl.ds(g, buf.shape[2] // _GROUPS, stride=_GROUPS)
        words = jnp.concatenate([buf[a, s, every, :] for a, s in regions], axis=0)
        return pltpu.bitcast(words, bf16)

    def rows_of(g):
        return pl.ds(pl.multiple_of(g * group_rows, group_rows), group_rows)

    x_copy = pltpu.make_async_copy(x_hbm, x_buf, small_sem.at[0])
    wr_copy = pltpu.make_async_copy(wr_hbm, wr_buf, small_sem.at[1])
    x_copy.start()
    wr_copy.start()
    queue_until(2)

    spread = _one_hot(_iota((_LANES, wide), 1) // slots == _iota((_LANES, wide), 0))

    def batch_major(row):
        g, slot = row // group_rows, (row // batch) % slots
        head = (slot // 2) * (2 * _GROUPS) + 2 * g + slot % 2
        return (row % batch) * heads + head

    by_batch = _one_hot(_iota((rows, rows), 0) == batch_major(_iota((rows, rows), 1)))
    by_group = _one_hot(_iota((rows, rows), 1) == batch_major(_iota((rows, rows), 0)))

    def own_slot(v):
        keep = (_iota(v.shape, 0) // batch) % slots == _iota(v.shape, 1) % slots
        return jnp.where(keep, v, 0.0).astype(bf16)

    y_buf[...] = jnp.zeros_like(y_buf)
    x_copy.wait()
    wr_copy.wait()
    x = x_buf[...].astype(f32)
    mean = jnp.mean(x, axis=-1, keepdims=True)
    var = jnp.mean(jnp.square(x - mean), axis=-1, keepdims=True)
    xn_bf = ((x - mean) / jnp.sqrt(var + 1e-5)).astype(bf16)
    xn = xn_bf.astype(f32)
    w_r = wr_buf[...].astype(f32).reshape(1, model)
    route = jax.nn.sigmoid(jnp.sum(xn * w_r, axis=-1, keepdims=True))
    xn_rows = jnp.concatenate([xn, xn], axis=0)
    xn_rows = jnp.concatenate([xn_rows] * (slots // 2), axis=0).astype(bf16)
    for k0 in range(0, model, _LANES):
        n = min(_LANES, model - k0)
        xn_buf[:, slots * k0:slots * (k0 + n)] = own_slot(
            _dot(xn_rows[:, k0:k0 + n], spread[:n, :slots * n], _NN))

    def ffn_block(j):
        _wait_filled(ff_buf.at[pl.ds(3 * j * ff_pieces, 3 * ff_pieces)], ff_sem.at[j])
        gate, up, down = (slab(ff_buf, (3 * j + m) * ff_pieces, ff_pieces) for m in range(3))
        hidden = jax.nn.silu(_dot(xn_bf, gate, _NN)) * _dot(xn_bf, up, _NN)
        y_buf[...] += _dot(hidden.astype(bf16), down, _NT)

    def query(g):
        q_buf[g] = _dot(xn_buf[...], head_group(wq_buf, g), _NN).astype(bf16)

    def absorb(g):
        z = _dot(q_buf[g], head_group(wuk_buf, g), _NT)
        wide_buf[rows_of(g), :] = own_slot(z * head_dim ** -0.5)

    queue_until(wq_end + _LAG - 2)
    ffn_block(0)
    queue_until(wq_end + _LAG)
    _wait_filled(wq_buf, w_sem.at[0])
    query(0)
    steps(_GROUPS - 1, lambda i, _: query(i + 1))
    queue_until(wuk_end + _LAG - 2)
    ffn_block(1)
    queue_until(wuk_end + _LAG)
    _wait_filled(wuk_buf, w_sem.at[1])
    pl.loop(0, _GROUPS // 2)(absorb)
    steps(1)
    pl.loop(_GROUPS // 2, _GROUPS)(absorb)
    for k in range(latent // _LANES):
        if k % 2 == 0:
            steps(1)
        part = _dot(wide_buf[:, k * wide:(k + 1) * wide], spread, _NT).astype(bf16)
        qa_buf[:, k * _LANES:(k + 1) * _LANES] = _dot(by_batch, part, _NN).astype(bf16)

    def attend(j, carry, new, old, top):
        new_top, total, acc = carry
        keys = pl.ds(pl.multiple_of(j * _KEYS, _KEYS), _KEYS)
        if old is not None:
            p = jnp.exp(s_buf[old % 2, :, keys] - top)
            for k0 in range(0, _KEYS, _LANES):
                total = total + p[:, k0:k0 + _LANES]
            values = slab(kv_buf, (old * chunks + j) * kv_pieces, kv_pieces)
            acc = acc + _dot(p.astype(bf16), values, _NN)
        if new is not None:
            u = new * chunks + j
            _wait_filled(kv_buf.at[pl.ds(u * kv_pieces, kv_pieces)], kv_sem.at[u])
            s = _dot(qa_buf[pl.ds(new * heads, heads), :],
                     slab(kv_buf, u * kv_pieces, kv_pieces), _NT)
            s_buf[new % 2, :, keys] = s
            for k0 in range(0, _KEYS, _LANES):
                new_top = jnp.maximum(new_top, s[:, k0:k0 + _LANES])
        return new_top, total, acc

    top = None
    for b in range(batch + 1):
        new = b if b < batch else None
        old = b - 1 if b > 0 else None
        chunk = functools.partial(attend, new=new, old=old, top=top)
        per = 2 if old is None else (chunks // 2 if new is None else 1)

        def some_chunks(i, carry, chunk=chunk, per=per):
            return jax.lax.fori_loop(i * per, (i + 1) * per, chunk, carry)

        new_top, total, acc = steps(chunks // per, chunk if per == 1 else some_chunks, (
            None if new is None else jnp.full((heads, _LANES), -jnp.inf, f32),
            None if old is None else jnp.zeros((heads, _LANES), f32),
            None if old is None else jnp.zeros((heads, latent), f32)))
        if old is not None:
            lat = acc / jnp.sum(total, axis=-1, keepdims=True)
            lat_buf[pl.ds(old * heads, heads), :] = lat.astype(bf16)
        if new is not None:
            top = jnp.max(new_top, axis=-1, keepdims=True)
            ffn_block(2 + b)

    def context(g):
        ctx = _dot(wide_buf[rows_of(g), :], head_group(wuv_buf, g), _NN)
        odd = _iota((2 * batch, head_dim), 0) >= batch
        for p in range(slots // 2):
            pair = ctx[2 * batch * p:2 * batch * (p + 1)]
            head = 2 * _GROUPS * p + 2 * g
            ctx_buf[head] = jnp.where(odd, 0.0, pair).astype(bf16)
            ctx_buf[head + 1] = jnp.where(odd, pair, 0.0).astype(bf16)

    steps(1)
    lat = _dot(by_group, lat_buf[...], _NN).astype(bf16)
    for k in range(latent // _LANES):
        wide_buf[:, k * wide:(k + 1) * wide] = own_slot(
            _dot(lat[:, k * _LANES:(k + 1) * _LANES], spread, _NN))
    steps(1)
    ffn_block(6)
    queue_until(wuv_end + _LAG)
    _wait_filled(wuv_buf, w_sem.at[2])
    pl.loop(0, _GROUPS // 2)(context)
    steps(1)
    pl.loop(_GROUPS // 2, _GROUPS)(context)

    def project(block, halves, parts):
        parts = [(part & 3, part >> 2, wo_sem.at[block, part]) for part in parts]

        def rows_at(k):
            return pl.ds(k * head_words + 2 * block * _WORDS, halves * _WORDS)

        for s, k, sem in parts:
            _wait_filled(wo_buf.at[:, s, rows_at(k)], sem)
        sides = range(_REGIONS[0])
        ctx = jnp.concatenate(
            [ctx_buf[(a * _REGIONS[1] + s) * 4 + k] for s, k, _ in parts for a in sides], axis=1)
        w_o = jnp.concatenate(
            [pltpu.bitcast(wo_buf[a, s, rows_at(k), :], bf16) for s, k, _ in parts for a in sides],
            axis=1)
        return _dot(ctx, w_o, _NT)

    queue_until(max(queued[0] + 1, narrow_end + _LAG))
    ffn_block(7)
    narrow = project(full_blocks, 1, range(16))
    blocks = []
    for block in range(full_blocks - 1):
        queue_until(max(queued[0] + 1, narrow_end + 2 * (block + 1) + _LAG))
        if block == full_blocks - 2:
            ffn_block(8)
        blocks.append(project(block, 2, range(16)))
    assert queued[0] == last_unit
    gate = jax.nn.silu(xn + (xn * 0.0 + y_buf[...] * route))

    def emit(first, acc):
        cols = slice(first, first + acc.shape[1])
        attn = acc[:batch] + acc[batch:]
        o_ref[:, cols] = (x[:, cols] + attn * gate[:, cols]).astype(o_ref.dtype)

    emit(0, jnp.concatenate(blocks, axis=1))
    emit(full_blocks * _LANES, narrow)
    acc = project(full_blocks - 1, 2, range(4))
    for lo, hi in ((4, 8), (8, 12), (12, 14), (14, 16)):
        acc = acc + project(full_blocks - 1, 2, range(lo, hi))
    emit((full_blocks - 1) * _LANES, acc)


@jax.jit
def pallas_recurrent_scan__compressed_kv_cla__moe_arch_mod__decode_kernel(
    A_x: jax.Array,
    A_c_kv: jax.Array,
    A_w_q: jax.Array,
    A_w_uk: jax.Array,
    A_w_uv: jax.Array,
    A_w_o: jax.Array,
    B_x: jax.Array,
    B_w_r: jax.Array,
    B_w_gate: jax.Array,
    B_w_up: jax.Array,
    B_w_down: jax.Array,
):
    del B_x
    batch, _, model = A_x.shape
    _, seq, latent = A_c_kv.shape
    _, heads, head_dim = A_w_q.shape
    hidden = B_w_gate.shape[1]
    parts = _REGIONS[0] * _REGIONS[1]
    slots = heads // _GROUPS
    f32, bf16, u32 = jnp.float32, jnp.bfloat16, jnp.uint32
    vmem, dma = pltpu.VMEM, pltpu.SemaphoreType.DMA

    def by_region(w):
        return w.reshape(*_REGIONS, -1, head_dim)

    def by_piece(w):
        return w.reshape(model // _ROWS, _ROWS, hidden)

    def words(n):
        return vmem((*_REGIONS, n * heads // (2 * parts), head_dim), u32)

    out = pl.pallas_call(
        _kernel,
        in_specs=[pl.BlockSpec(memory_space=pl.ANY)] * 10,
        out_specs=pl.BlockSpec(memory_space=pltpu.VMEM),
        out_shape=jax.ShapeDtypeStruct((batch, model), A_x.dtype),
        scratch_shapes=[
            vmem((batch, model), bf16),
            vmem((model,), bf16),
            vmem((batch * seq // _ROWS, _ROWS, latent), bf16),
            vmem((3 * (hidden // latent) * (model // _ROWS), _ROWS, latent), bf16),
            words(model), words(latent), words(latent), words(model),
            vmem((slots * batch, slots * model), bf16),
            vmem((_GROUPS, slots * batch, head_dim), bf16),
            vmem((batch * heads, slots * latent), bf16),
            vmem((batch * heads, latent), bf16),
            vmem((2, heads, seq), f32),
            vmem((batch * heads, latent), bf16),
            vmem((heads, 2 * batch, head_dim), bf16),
            vmem((batch, model), f32),
            dma((2,)),
            dma((3,)),
            dma((batch * seq // _KEYS,)),
            dma((pl.cdiv(model, _LANES), heads // _REGIONS[0])),
            dma((hidden // latent,)),
        ],
        compiler_params=pltpu.CompilerParams(
            vmem_limit_bytes=100 * 1024 * 1024,
            disable_semaphore_checks=True,
            disable_bounds_checks=True,
        ),
    )(
        A_x.reshape(batch, model),
        A_c_kv.reshape(batch, *_REGIONS, seq // (parts * _ROWS), _ROWS, latent),
        by_region(A_w_q),
        by_region(A_w_uk),
        by_region(A_w_uv),
        by_region(jnp.transpose(A_w_o, (0, 2, 1))),
        B_w_r,
        by_piece(B_w_gate),
        by_piece(B_w_up),
        by_piece(B_w_down.T),
    )
    return out.reshape(A_x.shape)
```
